```python
import jax
import jax.numpy as jnp

def _softmax(x, axis=-1):
    return jax.nn.softmax(x, axis=axis)
def _gelu(x):
    return jax.nn.gelu(x, approximate=True)
def _silu(x):
    return jax.nn.silu(x)
def _sigmoid(x):
    return jax.nn.sigmoid(x)
def _layernorm(x, axis=-1, eps=1e-5):
    m = jnp.mean(x, axis=axis, keepdims=True)
    v = jnp.var(x, axis=axis, keepdims=True)
    return (x - m) / jnp.sqrt(v + eps)
def _scatter_add(tgt, idx, src, axis=0):
    return tgt.at[idx].add(src)
def _segment_sum(src, seg, n):
    return jax.ops.segment_sum(src, seg, n)
class _Rng:
    def __init__(self, key):
        self._k = key
    def _next(self):
        self._k, sub = jax.random.split(self._k)
        return sub
    def normal(self, shape):
        return jax.random.normal(self._next(), shape, dtype=jnp.bfloat16)
    def randint(self, lo, hi, shape):
        return jax.random.randint(self._next(), shape, lo, hi, dtype=jnp.int32)
    def uniform(self, shape, lo=0.0, hi=1.0):
        return jax.random.uniform(self._next(), shape, jnp.bfloat16, lo, hi)
    def permutation(self, n):
        return jax.random.permutation(self._next(), n)


kernel_name = 'standalone__batchnorm__prompt'

def setup_inputs():
    _rng = _Rng(jax.random.key(int.from_bytes(__import__("os").urandom(4), "little")))
    _w = (lambda a: (lambda t: t.astype(jnp.bfloat16) if jnp.issubdtype(t.dtype, jnp.floating) else t)(jnp.asarray(a)))
    B, S, C = 2, 2048, 1024
    K = 3
    return {
        "x": _w((lambda *s: _rng.normal(s) * 0.05)(B, S, C)),
        "w": _w((lambda *s: _rng.normal(s) * 0.05)(K, C, C) * (1.0 / (K * C) ** 0.5)),
        "mean": _w((lambda *s: _rng.normal(s) * 0.05)(C) * 0.1),
        "var": _w(jnp.abs((lambda *s: _rng.normal(s) * 0.05)(C)) + 0.5),
        "g": _w((lambda *s: _rng.normal(s) * 0.05)(C) + 1.0),
        "b": _w((lambda *s: _rng.normal(s) * 0.05)(C) * 0.1),
    }

def reference(x, w, mean, var, g, b):
    K = 3
    P = K // 2
    S = x.shape[1]
    xp = jnp.pad(x, ((0, 0), (P, P), (0, 0)))
    y = sum(jnp.einsum('bsc,cd->bsd', xp[:, k:k + S, :], w[k]) for k in range(K))
    inv_std = 1.0 / jnp.sqrt(var + 1e-5)
    y = (y - mean) * (g * inv_std) + b
    return _silu(y)
```

```python
import jax
import jax.numpy as jnp
from jax import lax
import jax.experimental.pallas as pl
import jax.experimental.pallas.tpu as pltpu

_A, _B = 0.5, 2.0
_A2, _B2 = _A * _A, _B * _B
_NA = 2.0 * _A2 * (_A2 - _B2)
_NB = 2.0 * _B2 * (_B2 - _A2)
_EPS = 1e-5

_H = 8
_GT = 128
_KS = 128
_UNROLL = 2
_ORDER = (0, 5, 1, 3, 2, 4)
_LAST_SLABS = (512, 384, 128)


def _kernel(x_hbm, w_hbm, mean_hbm, var_hbm, g_hbm, b_hbm, o_hbm,
            xbuf, g0b, g5b, gpb, w1b, obuf, acc, pbuf, p_mean, p_var, p_g, p_b,
            ssem, xsem, psem, osem):
    f32, u32, bf16 = jnp.float32, jnp.uint32, jnp.bfloat16
    B, S, C = x_hbm.shape
    S2, C2, NC = S // 2, C // 2, C // 128
    H, gt = _H, _GT
    m = 2 * gt
    per = S2 // m
    NT = B * per
    nks = C // _KS

    xh = x_hbm.bitcast(u32)
    wh = w_hbm.bitcast(u32)
    oh = o_hbm.bitcast(u32)

    tobf = lambda v: pltpu.bitcast(v, bf16)
    lo32 = lambda v: pltpu.unpack_elementwise(v, index=0, packed_dtype=bf16, unpacked_dtype=f32)
    hi32 = lambda v: pltpu.unpack_elementwise(v, index=1, packed_dtype=bf16, unpacked_dtype=f32)
    pack = lambda lo, hi: pltpu.bitcast(pltpu.pack_elementwise([lo, hi], packed_dtype=bf16), u32)
    dot = lambda l, r: jnp.dot(l, r, preferred_element_type=f32)

    def chunk_rows(i):
        t = i % per
        lo = 0 if t == 0 else t * m + H
        hi = S2 if t == per - 1 else (t + 1) * m + H
        return i // per, lo, hi - lo

    def x_copy(i, c, sem):
        bi, lo, n = chunk_rows(i)
        return pltpu.make_async_copy(xh.at[bi, pl.ds(lo, n), pl.ds(c * 128, 128)],
                                     xbuf.at[bi, c, pl.ds(H + lo, n), :], sem)

    def slice_copies(s):
        r = pl.ds(s * _KS // 2, _KS // 2)
        cps = [x_copy(0, c, ssem.at[s]) for c in range(s * _KS // 128, (s + 1) * _KS // 128)]
        cps += [pltpu.make_async_copy(wh.at[0, r, :], g0b.at[r, :], ssem.at[s]),
                pltpu.make_async_copy(wh.at[2, r, :], g5b.at[r, :], ssem.at[s]),
                pltpu.make_async_copy(wh.at[1, r, :], w1b.at[r, :], ssem.at[s])]
        return cps

    p_copies = [pltpu.make_async_copy(src, dst, psem.at[i]) for i, (src, dst) in enumerate(
        ((mean_hbm, p_mean), (var_hbm, p_var), (g_hbm, p_g), (b_hbm, p_b)))]

    def o_copy(i, c, bi, r0):
        return pltpu.make_async_copy(obuf.at[i, c, pl.ds(0, m), :],
                                     oh.at[bi, pl.ds(r0, m), pl.ds(c * 128, 128)], osem.at[0])

    def wait_chunk(i):
        t = i % per
        for cond, n in ((t == 0, m + H), (t == per - 1, m - H),
                        (jnp.logical_and(t > 0, t < per - 1), m)):
            @pl.when(cond)
            def _(n=n):
                d = xbuf.at[0, :, pl.ds(0, n), :]
                pltpu.make_async_copy(d, d, xsem.at[i]).wait()

    all_cols = tuple(range(NC))

    def ldw(bi, r0, off, cols):
        vs = [xbuf[bi, c, pl.ds(r0 + H + off, gt, stride=2), :] for c in cols]
        return vs[0] if len(vs) == 1 else jnp.concatenate(vs, axis=1)

    def T0(bi, r0, cols=all_cols):
        E, O, Op = ldw(bi, r0, 0, cols), ldw(bi, r0, 1, cols), ldw(bi, r0, -1, cols)
        return ((hi32(O) + hi32(Op)) - (_A2 + _B2) * hi32(E)).astype(bf16)

    def T5(bi, r0, cols=all_cols):
        E, O, En = ldw(bi, r0, 0, cols), ldw(bi, r0, 1, cols), ldw(bi, r0, 2, cols)
        return ((lo32(En) + lo32(E)) - (_A2 + _B2) * lo32(O)).astype(bf16)

    def Tpair(bi, r0, which, cols=all_cols):
        E, O = ldw(bi, r0, 0, cols), ldw(bi, r0, 1, cols)
        d1, d2, d3, d4 = lo32(E), hi32(E), lo32(O), hi32(O)
        p, q2 = (_A, _B2) if which == 0 else (_B, _A2)
        e = d4 - q2 * d2
        o = (d3 - q2 * d1) * p
        return (e + o).astype(bf16), (e - o).astype(bf16)

    def g_transform(r, n):
        w0_, w1_, w2_ = g0b[r:r + n, :], w1b[r:r + n, :], g5b[r:r + n, :]
        outs = ([], [], [], [])
        for un in (lo32, hi32):
            u0, u1, u2 = un(w0_), un(w1_), un(w2_)
            ea = u0 * (1.0 / _NA) + u2 * (_A2 / _NA)
            oa = u1 * (_A / _NA)
            eb = u0 * (1.0 / _NB) + u2 * (_B2 / _NB)
            ob = u1 * (_B / _NB)
            for k, v in enumerate((ea + oa, ea - oa, eb + ob, eb - ob)):
                outs[k].append(v)
        for j in range(4):
            gpb[j, r:r + n, :] = pack(*outs[j])

    def G(j, r, c):
        return tobf(g0b[r, c] if j == 0 else g5b[r, c] if j == 5 else gpb[j - 1, r, c])

    def output(i, bi, r0, M, c0, c1):
        Sa, Da = M[1] + M[2], M[1] - M[2]
        Sb, Db = M[3] + M[4], M[3] - M[4]
        y0 = M[0] + Sa + Sb
        y1 = _A * Da + _B * Db
        y2 = _A2 * Sa + _B2 * Sb
        y3 = (_A * _A2) * Da + (_B * _B2) * Db + M[5]
        hs, hb = pbuf[0:1, c0:c1], pbuf[1:2, c0:c1]

        def act(y):
            h = y * hs + hb
            return h + h * jnp.tanh(h)

        ev, od = pack(act(y0), act(y1)), pack(act(y2), act(y3))
        for c in range(c0 // 128, c1 // 128):
            lanes = slice(c * 128 - c0, (c + 1) * 128 - c0)
            obuf[i, c, pl.ds(0, gt, stride=2), :] = ev[:, lanes]
            obuf[i, c, pl.ds(1, gt, stride=2), :] = od[:, lanes]
        for c in range(c0 // 128, c1 // 128):
            o_copy(i, c, bi, r0).start()

    def tile(i, bi, r0, slabs):
        T = {}
        c0 = 0
        for nc in slabs:
            c1 = c0 + nc
            M = {}
            for j in _ORDER:
                if j not in T:
                    if j == 0:
                        T[0] = T0(bi, r0)
                    elif j == 5:
                        T[5] = T5(bi, r0)
                    else:
                        k = (j - 1) // 2
                        T[1 + 2 * k], T[2 + 2 * k] = Tpair(bi, r0, k)
                M[j] = dot(T[j], G(j, slice(None), slice(c0, c1)))
            output(i, bi, r0, M, c0, c1)
            c0 = c1

    SC = [slice_copies(s) for s in range(nks)]
    for cps in SC:
        for cp in cps:
            cp.start()
    for cp in p_copies:
        cp.start()
    for c in range(NC):
        x_copy(1, c, xsem.at[1]).start()
    for bi in range(B):
        xbuf[bi, :, 0:H, :] = jnp.zeros((NC, H, 128), u32)
        xbuf[bi, :, H + S2:H + S2 + H, :] = jnp.zeros((NC, H, 128), u32)

    M = {}
    for s in range(nks):
        final = s == nks - 1
        for cp in SC[s]:
            cp.wait()
        if final:
            for cp in p_copies:
                cp.wait()
            for i in range(2, NT):
                for c in range(NC):
                    x_copy(i, c, xsem.at[i]).start()
            ld = lambda r: r[...].astype(f32).reshape(1, C)
            scale = ld(p_g) * lax.rsqrt(ld(p_var) + _EPS)
            pbuf[0:1, :] = 0.5 * scale
            pbuf[1:2, :] = 0.5 * (ld(p_b) - ld(p_mean) * scale)
        cols = tuple(range(s * _KS // 128, (s + 1) * _KS // 128))
        rr = slice(s * _KS // 2, (s + 1) * _KS // 2)
        part = {0: dot(T0(0, 0, cols), G(0, rr, slice(None))),
                5: dot(T5(0, 0, cols), G(5, rr, slice(None)))}
        g_transform(s * _KS // 2, _KS // 2)
        for k in range(2):
            ta, tb = Tpair(0, 0, k, cols)
            part[1 + 2 * k] = dot(ta, G(1 + 2 * k, rr, slice(None)))
            part[2 + 2 * k] = dot(tb, G(2 + 2 * k, rr, slice(None)))
        for j in range(6):
            d = part[j] if s == 0 else part[j] + acc[j]
            if final:
                M[j] = d
            else:
                acc[j] = d
    output(0, 0, 0, M, 0, C)

    def body(ii, carry):
        for u in range(_UNROLL):
            wait_chunk(1 + ii * _UNROLL + u)
        for u in range(_UNROLL):
            i = 1 + ii * _UNROLL + u
            tile(i, i // per, pl.multiple_of((i % per) * m, m), (C,))
        return carry

    lax.fori_loop(0, (NT - 2) // _UNROLL, body, 0)

    for c in range(NC):
        x_copy(NT - 1, c, xsem.at[NT - 1]).wait()
    tile(NT - 1, (NT - 1) // per, ((NT - 1) % per) * m, _LAST_SLABS)

    ov = obuf.at[:, :, pl.ds(0, m), :]
    pltpu.make_async_copy(ov, ov, osem.at[0]).wait()


@jax.jit
def pallas_standalone__batchnorm__prompt_kernel(
    x: jax.Array,
    w: jax.Array,
    mean: jax.Array,
    var: jax.Array,
    g: jax.Array,
    b: jax.Array,
):
    B, S, C = x.shape
    u32, f32 = jnp.uint32, jnp.float32
    m = 2 * _GT
    NT = B * (S // 2) // m
    NC = C // 128
    assert w.shape == (3, C, C) and x.dtype == jnp.bfloat16 and w.dtype == jnp.bfloat16
    assert S % (2 * m) == 0 and C % 128 == 0 and sum(_LAST_SLABS) == C
    assert (NT - 2) % _UNROLL == 0 and (S // 2) // m >= 2

    any_spec = pl.BlockSpec(memory_space=pl.ANY)
    return pl.pallas_call(
        _kernel,
        out_shape=jax.ShapeDtypeStruct((B, S, C), x.dtype),
        in_specs=[any_spec] * 6,
        out_specs=any_spec,
        scratch_shapes=[
            pltpu.VMEM((B, NC, S // 2 + 2 * _H, 128), u32),
            pltpu.VMEM((C // 2, C), u32),
            pltpu.VMEM((C // 2, C), u32),
            pltpu.VMEM((4, C // 2, C), u32),
            pltpu.VMEM((C // 2, C), u32),
            pltpu.VMEM((NT, NC, m + 8, 128), u32),
            pltpu.VMEM((6, _GT, C), f32),
            pltpu.VMEM((8, C), f32),
            pltpu.VMEM((C,), mean.dtype), pltpu.VMEM((C,), var.dtype),
            pltpu.VMEM((C,), g.dtype), pltpu.VMEM((C,), b.dtype),
            pltpu.SemaphoreType.DMA((C // _KS,)),
            pltpu.SemaphoreType.DMA((NT,)),
            pltpu.SemaphoreType.DMA((4,)),
            pltpu.SemaphoreType.DMA((1,)),
        ],
        compiler_params=pltpu.CompilerParams(vmem_limit_bytes=100 * 1024 * 1024),
    )(x, w, mean, var, g, b)
```

```python
import jax
import jax.numpy as jnp
from jax import lax
import jax.experimental.pallas as pl
import jax.experimental.pallas.tpu as pltpu

_A, _B = 0.5, 2.0
_A2, _B2 = _A * _A, _B * _B
_NA = 2.0 * _A2 * (_A2 - _B2)
_NB = 2.0 * _B2 * (_B2 - _A2)
_EPS = 1e-5

_H = 8
_GT = 128
_KS = 128
_UNROLL = 2
_ORDER = (0, 5, 1, 3, 2, 4)
_LAST_SLABS = (512, 384, 128)


def _kernel(x_hbm, w_hbm, mean_hbm, var_hbm, g_hbm, b_hbm, o_hbm,
            xbuf, g0b, g5b, gpb, w1b, obuf, acc, pbuf, p_mean, p_var, p_g, p_b,
            ssem, xsem, psem, osem):
    f32, u32, bf16 = jnp.float32, jnp.uint32, jnp.bfloat16
    B, S, C = x_hbm.shape
    S2, C2, NC = S // 2, C // 2, C // 128
    H, gt = _H, _GT
    m = 2 * gt
    per = S2 // m
    NT = B * per
    nks = C // _KS

    xh = x_hbm.bitcast(u32)
    wh = w_hbm.bitcast(u32)
    oh = o_hbm.bitcast(u32)

    tobf = lambda v: pltpu.bitcast(v, bf16)
    lo32 = lambda v: pltpu.bitcast(v << 16, f32)
    hi32 = lambda v: pltpu.bitcast(v & u32(0xFFFF0000), f32)
    rnd = lambda v: pltpu.bitcast(v.astype(bf16).astype(f32), u32)
    pack = lambda lo, hi: (rnd(lo) >> 16) | rnd(hi)
    dot = lambda l, r: jnp.dot(l, r, preferred_element_type=f32)

    def chunk_rows(i):
        t = i % per
        lo = 0 if t == 0 else t * m + H
        hi = S2 if t == per - 1 else (t + 1) * m + H
        return i // per, lo, hi - lo

    def x_copy(i, c, sem):
        bi, lo, n = chunk_rows(i)
        return pltpu.make_async_copy(xh.at[bi, pl.ds(lo, n), pl.ds(c * 128, 128)],
                                     xbuf.at[bi, c, pl.ds(H + lo, n), :], sem)

    def slice_copies(s):
        r = pl.ds(s * _KS // 2, _KS // 2)
        cps = [x_copy(0, c, ssem.at[s]) for c in range(s * _KS // 128, (s + 1) * _KS // 128)]
        cps += [pltpu.make_async_copy(wh.at[0, r, :], g0b.at[r, :], ssem.at[s]),
                pltpu.make_async_copy(wh.at[2, r, :], g5b.at[r, :], ssem.at[s]),
                pltpu.make_async_copy(wh.at[1, r, :], w1b.at[r, :], ssem.at[s])]
        return cps

    p_copies = [pltpu.make_async_copy(src, dst, psem.at[i]) for i, (src, dst) in enumerate(
        ((mean_hbm, p_mean), (var_hbm, p_var), (g_hbm, p_g), (b_hbm, p_b)))]

    def o_copy(i, c, bi, r0):
        return pltpu.make_async_copy(obuf.at[i, c, pl.ds(0, m), :],
                                     oh.at[bi, pl.ds(r0, m), pl.ds(c * 128, 128)], osem.at[0])

    def wait_chunk(i):
        t = i % per
        for cond, n in ((t == 0, m + H), (t == per - 1, m - H),
                        (jnp.logical_and(t > 0, t < per - 1), m)):
            @pl.when(cond)
            def _(n=n):
                d = xbuf.at[0, :, pl.ds(0, n), :]
                pltpu.make_async_copy(d, d, xsem.at[i]).wait()

    all_cols = tuple(range(NC))

    def ldw(bi, r0, off, cols):
        vs = [xbuf[bi, c, pl.ds(r0 + H + off, gt, stride=2), :] for c in cols]
        return vs[0] if len(vs) == 1 else jnp.concatenate(vs, axis=1)

    def T0(bi, r0, cols=all_cols):
        E, O, Op = ldw(bi, r0, 0, cols), ldw(bi, r0, 1, cols), ldw(bi, r0, -1, cols)
        return ((hi32(O) + hi32(Op)) - (_A2 + _B2) * hi32(E)).astype(bf16)

    def T5(bi, r0, cols=all_cols):
        E, O, En = ldw(bi, r0, 0, cols), ldw(bi, r0, 1, cols), ldw(bi, r0, 2, cols)
        return ((lo32(En) + lo32(E)) - (_A2 + _B2) * lo32(O)).astype(bf16)

    def Tpair(bi, r0, which, cols=all_cols):
        E, O = ldw(bi, r0, 0, cols), ldw(bi, r0, 1, cols)
        d1, d2, d3, d4 = lo32(E), hi32(E), lo32(O), hi32(O)
        p, q2 = (_A, _B2) if which == 0 else (_B, _A2)
        e = d4 - q2 * d2
        o = (d3 - q2 * d1) * p
        return (e + o).astype(bf16), (e - o).astype(bf16)

    def g_transform(r, n):
        u0, u1, u2 = (tobf(ref[r:r + n, :]).astype(f32) for ref in (g0b, w1b, g5b))
        ea = u0 * (1.0 / _NA) + u2 * (_A2 / _NA)
        oa = u1 * (_A / _NA)
        eb = u0 * (1.0 / _NB) + u2 * (_B2 / _NB)
        ob = u1 * (_B / _NB)
        for j, v in enumerate((ea + oa, ea - oa, eb + ob, eb - ob)):
            gpb[j, r:r + n, :] = pltpu.bitcast(v.astype(bf16), u32)

    def G(j, r, c):
        return tobf(g0b[r, c] if j == 0 else g5b[r, c] if j == 5 else gpb[j - 1, r, c])

    def output(i, bi, r0, M, c0, c1):
        Sa, Da = M[1] + M[2], M[1] - M[2]
        Sb, Db = M[3] + M[4], M[3] - M[4]
        y0 = M[0] + Sa + Sb
        y1 = _A * Da + _B * Db
        y2 = _A2 * Sa + _B2 * Sb
        y3 = (_A * _A2) * Da + (_B * _B2) * Db + M[5]
        hs, hb = pbuf[0:1, c0:c1], pbuf[1:2, c0:c1]

        def act(y):
            h = y * hs + hb
            return h + h * jnp.tanh(h)

        ev, od = pack(act(y0), act(y1)), pack(act(y2), act(y3))
        for c in range(c0 // 128, c1 // 128):
            lanes = slice(c * 128 - c0, (c + 1) * 128 - c0)
            obuf[i, c, pl.ds(0, gt, stride=2), :] = ev[:, lanes]
            obuf[i, c, pl.ds(1, gt, stride=2), :] = od[:, lanes]
        for c in range(c0 // 128, c1 // 128):
            o_copy(i, c, bi, r0).start()

    def tile(i, bi, r0, slabs):
        T = {}
        c0 = 0
        for nc in slabs:
            c1 = c0 + nc
            M = {}
            for j in _ORDER:
                if j not in T:
                    if j == 0:
                        T[0] = T0(bi, r0)
                    elif j == 5:
                        T[5] = T5(bi, r0)
                    else:
                        k = (j - 1) // 2
                        T[1 + 2 * k], T[2 + 2 * k] = Tpair(bi, r0, k)
                M[j] = dot(T[j], G(j, slice(None), slice(c0, c1)))
            output(i, bi, r0, M, c0, c1)
            c0 = c1

    SC = [slice_copies(s) for s in range(nks)]
    for cps in SC:
        for cp in cps:
            cp.start()
    for cp in p_copies:
        cp.start()
    for c in range(NC):
        x_copy(1, c, xsem.at[1]).start()
    for bi in range(B):
        xbuf[bi, :, 0:H, :] = jnp.zeros((NC, H, 128), u32)
        xbuf[bi, :, H + S2:H + S2 + H, :] = jnp.zeros((NC, H, 128), u32)

    M = {}
    for s in range(nks):
        final = s == nks - 1
        for cp in SC[s]:
            cp.wait()
        if final:
            for cp in p_copies:
                cp.wait()
            for i in range(2, NT):
                for c in range(NC):
                    x_copy(i, c, xsem.at[i]).start()
            ld = lambda r: r[...].astype(f32).reshape(1, C)
            scale = ld(p_g) * lax.rsqrt(ld(p_var) + _EPS)
            pbuf[0:1, :] = 0.5 * scale
            pbuf[1:2, :] = 0.5 * (ld(p_b) - ld(p_mean) * scale)
        cols = tuple(range(s * _KS // 128, (s + 1) * _KS // 128))
        rr = slice(s * _KS // 2, (s + 1) * _KS // 2)
        part = {0: dot(T0(0, 0, cols), G(0, rr, slice(None))),
                5: dot(T5(0, 0, cols), G(5, rr, slice(None)))}
        g_transform(s * _KS // 2, _KS // 2)
        for k in range(2):
            ta, tb = Tpair(0, 0, k, cols)
            part[1 + 2 * k] = dot(ta, G(1 + 2 * k, rr, slice(None)))
            part[2 + 2 * k] = dot(tb, G(2 + 2 * k, rr, slice(None)))
        for j in range(6):
            d = part[j] if s == 0 else part[j] + acc[j]
            if final:
                M[j] = d
            else:
                acc[j] = d
    output(0, 0, 0, M, 0, C)

    def body(ii, carry):
        for u in range(_UNROLL):
            wait_chunk(1 + ii * _UNROLL + u)
        for u in range(_UNROLL):
            i = 1 + ii * _UNROLL + u
            tile(i, i // per, pl.multiple_of((i % per) * m, m), (C,))
        return carry

    lax.fori_loop(0, (NT - 2) // _UNROLL, body, 0)

    for c in range(NC):
        x_copy(NT - 1, c, xsem.at[NT - 1]).wait()
    tile(NT - 1, (NT - 1) // per, ((NT - 1) % per) * m, _LAST_SLABS)

    ov = obuf.at[:, :, pl.ds(0, m), :]
    pltpu.make_async_copy(ov, ov, osem.at[0]).wait()


@jax.jit
def pallas_standalone__batchnorm__prompt_kernel(
    x: jax.Array,
    w: jax.Array,
    mean: jax.Array,
    var: jax.Array,
    g: jax.Array,
    b: jax.Array,
):
    B, S, C = x.shape
    u32, f32 = jnp.uint32, jnp.float32
    m = 2 * _GT
    NT = B * (S // 2) // m
    NC = C // 128
    assert w.shape == (3, C, C) and x.dtype == jnp.bfloat16 and w.dtype == jnp.bfloat16
    assert S % (2 * m) == 0 and C % 128 == 0 and sum(_LAST_SLABS) == C
    assert (NT - 2) % _UNROLL == 0 and (S // 2) // m >= 2

    any_spec = pl.BlockSpec(memory_space=pl.ANY)
    return pl.pallas_call(
        _kernel,
        out_shape=jax.ShapeDtypeStruct((B, S, C), x.dtype),
        in_specs=[any_spec] * 6,
        out_specs=any_spec,
        scratch_shapes=[
            pltpu.VMEM((B, NC, S // 2 + 2 * _H, 128), u32),
            pltpu.VMEM((C // 2, C), u32),
            pltpu.VMEM((C // 2, C), u32),
            pltpu.VMEM((4, C // 2, C), u32),
            pltpu.VMEM((C // 2, C), u32),
            pltpu.VMEM((NT, NC, m + 8, 128), u32),
            pltpu.VMEM((6, _GT, C), f32),
            pltpu.VMEM((8, C), f32),
            pltpu.VMEM((C,), mean.dtype), pltpu.VMEM((C,), var.dtype),
            pltpu.VMEM((C,), g.dtype), pltpu.VMEM((C,), b.dtype),
            pltpu.SemaphoreType.DMA((C // _KS,)),
            pltpu.SemaphoreType.DMA((NT,)),
            pltpu.SemaphoreType.DMA((4,)),
            pltpu.SemaphoreType.DMA((1,)),
        ],
        compiler_params=pltpu.CompilerParams(vmem_limit_bytes=100 * 1024 * 1024),
    )(x, w, mean, var, g, b)
```
